```python
import os as _os
_os.environ.setdefault("JAX_PLATFORMS", "cpu")
import jax
import jax.numpy as jnp

def _softmax(x, axis=-1):
    return jax.nn.softmax(x, axis=axis)
def _gelu(x):
    return jax.nn.gelu(x, approximate=True)
def _silu(x):
    return jax.nn.silu(x)
def _sigmoid(x):
    return jax.nn.sigmoid(x)
def _layernorm(x, axis=-1, eps=1e-5):
    m = jnp.mean(x, axis=axis, keepdims=True)
    v = jnp.var(x, axis=axis, keepdims=True)
    return (x - m) / jnp.sqrt(v + eps)
def _scatter_add(tgt, idx, src, axis=0):
    return tgt.at[idx].add(src)
def _segment_sum(src, seg, n):
    return jax.ops.segment_sum(src, seg, n)
class _Rng:
    def __init__(self, key):
        self._k = key
    def _next(self):
        self._k, sub = jax.random.split(self._k)
        return sub
    def normal(self, shape):
        return jax.random.normal(self._next(), shape, dtype=jnp.bfloat16)
    def randint(self, lo, hi, shape):
        return jax.random.randint(self._next(), shape, lo, hi, dtype=jnp.int32)
    def uniform(self, shape, lo=0.0, hi=1.0):
        return jax.random.uniform(self._next(), shape, jnp.bfloat16, lo, hi)
    def permutation(self, n):
        return jax.random.permutation(self._next(), n)


kernel_name = 'standalone__mha_block_cached__near_ridge'

def setup_inputs():
    _rng = _Rng(jax.random.key(int.from_bytes(__import__("os").urandom(4), "little")))
    _w = (lambda a: (lambda t: t.astype(jnp.bfloat16) if jnp.issubdtype(t.dtype, jnp.floating) else t)(jnp.asarray(a)))
    B, Sq, D = 8, 112, 640
    H, Sk, Dh = 32, 512, 192
    return {
        "x": _w((lambda *s: _rng.normal(s) * 0.8)(B, Sq, D)),
        "k_cache": _w((lambda *s: _rng.normal(s) * 0.8)(B, H, Sk, Dh)),
        "v_cache": _w((lambda *s: _rng.normal(s) * 0.05)(B, H, Sk, Dh)),
        "wq": _w((lambda *s: _rng.normal(s) * 0.8)(D, H * Dh) * (D ** -0.5)),
        "wo": _w((lambda *s: _rng.normal(s) * 0.05)(H * Dh, D) * ((H * Dh) ** -0.5)),
    }

def reference(x, k_cache, v_cache, wq, wo):
    B, Sq, D = x.shape
    H, Dh = 32, 192
    q = (lambda x, *d: x.transpose(*d))((x @ wq).reshape(B, Sq, H, Dh), 0, 2, 1, 3)
    scores = jnp.einsum("bhqd,bhkd->bhqk", q, k_cache) * (Dh ** -0.5)
    p = _softmax(scores, axis=-1)
    o = jnp.einsum("bhqk,bhkd->bhqd", p, v_cache)
    return (lambda x, *d: x.transpose(*d))(o, 0, 2, 1, 3).reshape(B, Sq, H * Dh) @ wo
```

```python
import jax
import jax.numpy as jnp
import jax.experimental.pallas as pl
import jax.experimental.pallas.tpu as pltpu

B, SQ, D = 8, 112, 640
H, SK, DH = 32, 512, 192
NG = H // 2
PW = 2 * DH
T = NG * B
NBUF = 8
U = 2
NBLK = T // U
KV_PRIO = 1
SCALE = (DH ** -0.5) * 1.4426950408889634
NT = (((1,), (1,)), ((), ()))
F32 = jnp.float32
BF16 = jnp.bfloat16


def _kernel(x_hbm, wq_hbm, kt_hbm, vt_hbm, wo_hbm, out_hbm,
            xbuf, wqbuf, wobuf, kbuf, vbuf,
            qa0, qb0, qa1, qb1, s0, s1, o0, o1, acc, obuf,
            ksem, vsem, wqsem, wosem, xsem, osem):
    qa = (qa0, qa1)
    qb = (qb0, qb1)
    ss = (s0, s1)
    oo = (o0, o1)

    def st(t):
        return isinstance(t, int)

    def grp(t):
        return t // B if st(t) else jax.lax.shift_right_logical(t, 3)

    def bat(t):
        return t % B if st(t) else jax.lax.bitwise_and(t, B - 1)

    def ring(t):
        return t % NBUF if st(t) else jax.lax.bitwise_and(t, NBUF - 1)

    def kcopy(t):
        sl = ring(t)
        return pltpu.make_async_copy(kt_hbm.at[bat(t), grp(t)], kbuf.at[sl], ksem.at[sl])

    def vcopy(t):
        sl = ring(t)
        return pltpu.make_async_copy(vt_hbm.at[bat(t), grp(t)], vbuf.at[sl], vsem.at[sl])

    def wqcopy(g):
        if st(g):
            src = wq_hbm.at[:, g * PW:(g + 1) * PW]
        else:
            src = wq_hbm.at[:, pl.ds(pl.multiple_of(g * PW, 128), PW)]
        return pltpu.make_async_copy(src, wqbuf.at[g], wqsem.at[g])

    def wocopy(g):
        return pltpu.make_async_copy(wo_hbm.at[g], wobuf.at[g], wosem.at[g])

    def xcopy(b):
        return pltpu.make_async_copy(x_hbm.at[b], xbuf.at[b], xsem.at[b])

    def ocopy(b):
        return pltpu.make_async_copy(obuf.at[b], out_hbm.at[b], osem.at[b])

    def when(cond, fn):
        if isinstance(cond, bool):
            if cond:
                fn()
        else:
            pl.when(cond)(fn)

    lane = jax.lax.broadcasted_iota(jnp.int32, (SQ, 256), 1)

    def qproj(t, sl):
        q = jnp.dot(xbuf[bat(t)], wqbuf[grp(t)], preferred_element_type=F32) * SCALE
        qa[sl][...] = jnp.where(lane < DH, q[:, 0:256], 0.0).astype(BF16)
        qb[sl][...] = jnp.where(lane >= 64, q[:, 128:384], 0.0).astype(BF16)

    def qk(t, sl):
        ks = ring(t)
        ss[sl][0] = jnp.dot(qa[sl][...], kbuf[ks, 0:256, :], preferred_element_type=F32)
        ss[sl][1] = jnp.dot(qb[sl][...], kbuf[ks, 128:384, :], preferred_element_type=F32)

    def softmax(sl):
        res = []
        for h in range(2):
            s = ss[sl][h]
            m = jnp.max(s, axis=-1, keepdims=True)
            p = jnp.exp2(s - m)
            l = jnp.sum(p, axis=-1, keepdims=True)
            res.append((p.astype(BF16), 1.0 / l))
        return res

    def pv(t, sl, res):
        vs = ring(t)
        (p0, r0), (p1, r1) = res
        ot0 = jax.lax.dot_general(vbuf[vs, 0:DH, :], p0, NT, preferred_element_type=F32)
        ot1 = jax.lax.dot_general(vbuf[vs, DH:PW, :], p1, NT, preferred_element_type=F32)
        o = jnp.concatenate([ot0, ot1], axis=0).T
        l384 = jax.lax.broadcasted_iota(jnp.int32, (SQ, PW), 1)
        o = o * jnp.where(l384 < DH, r0, r1)
        oo[sl][...] = o.astype(BF16)

    def outproj(t, sl):
        acc[bat(t)] += jnp.dot(oo[sl][...], wobuf[grp(t)], preferred_element_type=F32)

    def finalize(b):
        obuf[b] = acc[b].astype(BF16)
        ocopy(b).start()

    def weights_with_k(tk):
        when(jnp.logical_and(bat(tk + 3) == 0, tk + 3 < T) if not st(tk) else ((tk + 3) % B == 0 and tk + 3 < T),
             lambda: wqcopy(grp(tk + 3)).start())
        when(bat(tk) == 1, lambda: wocopy(grp(tk)).start())

    def step_waits(t):
        tk = t + 1
        when(tk < T, lambda: kcopy(tk).wait())
        vcopy(t).wait()
        tq = t + 2
        when(jnp.logical_and(bat(tq) == 0, tq < T) if not st(tq) else (tq % B == 0 and tq < T),
             lambda: wqcopy(grp(tq)).wait())
        to = t - 1
        when(bat(to) == 0, lambda: wocopy(grp(to)).wait())

    def sub(t, sl, do_qk=True, do_qp=True, do_op=True):
        res = softmax(sl)
        if do_qk:
            qk(t + 1, 1 - sl)
        if do_qp:
            qproj(t + 2, sl)
        pv(t, sl, res)
        if do_op:
            outproj(t - 1, 1 - sl)

    def waits(t0):
        for j in range(U):
            step_waits(t0 + j)

    def refill(t0):
        for j in range(U):
            tk = t0 + 1 + j + NBUF
            tv = t0 + j + NBUF

            def ik():
                kcopy(tk).start(priority=KV_PRIO)
                weights_with_k(tk)
            when(tk < T, ik)
            when(tv < T, lambda: vcopy(tv).start(priority=KV_PRIO))

    xcopy(0).start()
    wqcopy(0).start()
    kcopy(0).start(priority=KV_PRIO)
    xcopy(1).start()
    kcopy(1).start(priority=KV_PRIO)
    weights_with_k(1)
    vcopy(0).start(priority=KV_PRIO)
    for xb in range(2, B):
        xcopy(xb).start()
    for t in range(1, NBUF):
        if t + 1 < NBUF:
            kcopy(t + 1).start(priority=KV_PRIO)
            weights_with_k(t + 1)
        vcopy(t).start(priority=KV_PRIO)
    acc[...] = jnp.zeros_like(acc)
    xcopy(0).wait()
    wqcopy(0).wait()
    qproj(0, 0)
    kcopy(0).wait()
    xcopy(1).wait()
    qk(0, 0)
    qproj(1, 1)
    kcopy(NBUF).start(priority=KV_PRIO)
    weights_with_k(NBUF)
    for xb in range(2, B):
        xcopy(xb).wait()

    def block(t0, first=False, last=False):
        for j in range(U):
            sub(t0 + j, j % 2,
                do_qk=not (last and j == U - 1),
                do_qp=not (last and j >= U - 2),
                do_op=not (first and j == 0))

    waits(0)
    block(0, first=True)
    refill(0)
    waits(U)

    def body(i, c):
        t0 = i * U
        for j in range(U):
            tf = t0 - 2 - j
            when(tf >= T - B, lambda: finalize(bat(tf)))
        block(t0)
        refill(t0)
        waits(t0 + U)
        return c

    jax.lax.fori_loop(1, NBLK - 1, body, 0)

    t0 = T - U
    for j in range(U):
        tf = t0 - 2 - j
        if tf >= T - B:
            finalize(tf % B)
    block(t0, last=True)
    for tf in range(T - U - 1, T - 1):
        if tf >= T - B:
            finalize(tf % B)
    outproj(T - 1, (U - 1) % 2)
    finalize((T - 1) % B)
    for b in range(B):
        ocopy(b).wait()


@jax.jit
def pallas_standalone__mha_block_cached__near_ridge_kernel(x, k_cache, v_cache, wq, wo):
    kt = jnp.swapaxes(k_cache, 2, 3).reshape(B, NG, PW, SK)
    vt = jnp.swapaxes(v_cache, 2, 3).reshape(B, NG, PW, SK)
    wo3 = wo.reshape(NG, PW, D)
    return pl.pallas_call(
        _kernel,
        in_specs=[pl.BlockSpec(memory_space=pl.ANY)] * 5,
        out_specs=pl.BlockSpec(memory_space=pl.ANY),
        out_shape=jax.ShapeDtypeStruct((B, SQ, D), BF16),
        scratch_shapes=[
            pltpu.VMEM((B, SQ, D), BF16),
            pltpu.VMEM((NG, D, PW), BF16),
            pltpu.VMEM((NG, PW, D), BF16),
            pltpu.VMEM((NBUF, PW, SK), BF16),
            pltpu.VMEM((NBUF, PW, SK), BF16),
            pltpu.VMEM((SQ, 256), BF16), pltpu.VMEM((SQ, 256), BF16),
            pltpu.VMEM((SQ, 256), BF16), pltpu.VMEM((SQ, 256), BF16),
            pltpu.VMEM((2, SQ, SK), F32), pltpu.VMEM((2, SQ, SK), F32),
            pltpu.VMEM((SQ, PW), BF16), pltpu.VMEM((SQ, PW), BF16),
            pltpu.VMEM((B, SQ, D), F32),
            pltpu.VMEM((B, SQ, D), BF16),
            pltpu.SemaphoreType.DMA((NBUF,)),
            pltpu.SemaphoreType.DMA((NBUF,)),
            pltpu.SemaphoreType.DMA((NG,)),
            pltpu.SemaphoreType.DMA((NG,)),
            pltpu.SemaphoreType.DMA((B,)),
            pltpu.SemaphoreType.DMA((B,)),
        ],
        compiler_params=pltpu.CompilerParams(vmem_limit_bytes=64 * 1024 * 1024, disable_bounds_checks=True),
    )(x, wq, kt, vt, wo3)
```

```python
import jax
import jax.numpy as jnp
import jax.experimental.pallas as pl
import jax.experimental.pallas.tpu as pltpu

B, SQ, D = 8, 112, 640
H, SK, DH = 32, 512, 192
NG = H // 2
PW = 2 * DH
T = NG * B
NBUF = 8
DQ = 16
NQ = 16
NSINGLE = 8
XS = 4
HI, LO = 0, 1
SCALE = (DH ** -0.5) * 1.4426950408889634
NT = (((1,), (1,)), ((), ()))
F32 = jnp.float32
BF16 = jnp.bfloat16


def _kernel(x_hbm, wq_hbm, kt_hbm, vt_hbm, wo_hbm, out_hbm,
            xbuf, wqbuf, wobuf, kbuf, vbuf, qring,
            s0, s1, o0, o1, acc, obuf,
            ksem, vsem, wqsem, wosem, xsem, osem):
    ss = (s0, s1)
    oo = (o0, o1)

    def st(t):
        return isinstance(t, int)

    def grp(t):
        return t // B if st(t) else jax.lax.shift_right_logical(t, 3)

    def bat(t):
        return t % B if st(t) else jax.lax.bitwise_and(t, B - 1)

    def ring(t):
        return t % NBUF if st(t) else jax.lax.bitwise_and(t, NBUF - 1)

    def qslot(t):
        return t % NQ if st(t) else jax.lax.bitwise_and(t, NQ - 1)

    def when(cond, fn):
        if isinstance(cond, bool):
            if cond:
                fn()
        else:
            pl.when(cond)(fn)

    def land(a, b):
        if isinstance(a, bool) and isinstance(b, bool):
            return a and b
        return jnp.logical_and(a, b)

    def kcopy(t):
        sl = ring(t)
        return pltpu.make_async_copy(kt_hbm.at[bat(t), grp(t)], kbuf.at[sl], ksem.at[sl])

    def vcopy(t):
        sl = ring(t)
        return pltpu.make_async_copy(vt_hbm.at[bat(t), grp(t)], vbuf.at[sl], vsem.at[sl])

    def wqcopy(g):
        if st(g):
            src = wq_hbm.at[:, g * PW:(g + 1) * PW]
        else:
            src = wq_hbm.at[:, pl.ds(pl.multiple_of(g * PW, 128), PW)]
        return pltpu.make_async_copy(src, wqbuf.at[g], wqsem.at[g])

    def wocopy(g):
        return pltpu.make_async_copy(wo_hbm.at[g], wobuf.at[g], wosem.at[g])

    def xcopy(b):
        return pltpu.make_async_copy(x_hbm.at[b], xbuf.at[b], xsem.at[b])

    def ocopy(b):
        return pltpu.make_async_copy(obuf.at[b], out_hbm.at[b], osem.at[b])

    def arrival(buf, sem, idx):
        return pltpu.make_async_copy(buf.at[idx], buf.at[idx], sem.at[idx])

    lane = jax.lax.broadcasted_iota(jnp.int32, (SQ, 256), 1)

    def qproj(t):
        q = jnp.dot(xbuf[bat(t)], wqbuf[grp(t)], preferred_element_type=F32) * SCALE
        sl = qslot(t)
        qring[sl, 0] = jnp.where(lane < DH, q[:, 0:256], 0.0).astype(BF16)
        qring[sl, 1] = jnp.where(lane >= 64, q[:, 128:384], 0.0).astype(BF16)

    def qk(t, sl):
        ks = ring(t)
        qs = qslot(t)
        ss[sl][0] = jnp.dot(qring[qs, 0], kbuf[ks, 0:256, :], preferred_element_type=F32)
        ss[sl][1] = jnp.dot(qring[qs, 1], kbuf[ks, 128:384, :], preferred_element_type=F32)

    def softmax(sl):
        res = []
        for h in range(2):
            s = ss[sl][h]
            m = jnp.max(s, axis=-1, keepdims=True)
            p = jnp.exp2(s - m)
            l = jnp.sum(p, axis=-1, keepdims=True)
            res.append((p.astype(BF16), 1.0 / l))
        return res

    def pv(t, sl, res):
        vs = ring(t)
        (p0, r0), (p1, r1) = res
        ot0 = jax.lax.dot_general(vbuf[vs, 0:DH, :], p0, NT, preferred_element_type=F32)
        ot1 = jax.lax.dot_general(vbuf[vs, DH:PW, :], p1, NT, preferred_element_type=F32)
        o = jnp.concatenate([ot0, ot1], axis=0).T
        col = jax.lax.broadcasted_iota(jnp.int32, (SQ, PW), 1)
        oo[sl][...] = (o * jnp.where(col < DH, r0, r1)).astype(BF16)

    def outproj(t, sl):
        acc[bat(t)] += jnp.dot(oo[sl][...], wobuf[grp(t)], preferred_element_type=F32)

    def finalize(b, send):
        obuf[b] = acc[b].astype(BF16)
        if send:
            ocopy(b).start(priority=HI)

    def fin(tf):
        when(tf >= T - B, lambda: finalize(bat(tf), False))

    def step(t, sl, do_qk=True, do_qp=True):
        res = softmax(sl)
        if do_qk:
            qk(t + 1, 1 - sl)
        if do_qp:
            qproj(t + DQ)
        pv(t, sl, res)
        outproj(max(t - 1, 0) if st(t) else jnp.maximum(t - 1, 0), 1 - sl)

    def weights_with_k(tk):
        tq = tk + DQ
        when(land(bat(tq) == 0, tq < T), lambda: wqcopy(grp(tq)).start(priority=HI))
        to = tk - 1
        when(bat(to) == 0, lambda: wocopy(grp(to)).start(priority=HI))

    def waits(t0, par, u, with_qp):
        todo = []

        def add(cond, buf, sem, idx):
            if cond is not False:
                todo.append((cond, arrival(buf, sem, idx)))
        for j in range(u):
            t = t0 + j
            add(not (st(t) and t + 1 >= T), kbuf, ksem, ring(t + 1))
            add(True, vbuf, vsem, ring(t))
        for j in range(u):
            t = t0 + j
            if with_qp and (par + j + DQ) % 2 == 0:
                add(bat(t + DQ) == 0, wqbuf, wqsem, grp(t + DQ))
            if (par + j) % 2 == 1:
                add(bat(t - 1) == 0, wobuf, wosem, grp(t - 1))
        for c, cp in todo:
            when(c, cp.wait)

    def refill(t0, u):
        for j in range(u):
            tk = t0 + 1 + j + NBUF
            tv = t0 + j + NBUF

            def issue_k():
                weights_with_k(tk)
                kcopy(tk).start(priority=LO)
            when(tk < T, issue_k)
            when(tv < T, lambda: vcopy(tv).start(priority=LO))

    xcopy(0).start(priority=HI)
    wqcopy(0).start(priority=HI)
    for xb in range(1, B):
        xcopy(xb).start(priority=HI)
    kcopy(0).start(priority=LO)
    acc[...] = jnp.zeros_like(acc)
    o1[...] = jnp.zeros_like(o1)
    xcopy(0).wait()
    wqcopy(0).wait()
    for g in range(1, DQ // B + 1):
        wqcopy(g).start(priority=HI)
    for t in range(NBUF):
        if t + 1 < NBUF:
            weights_with_k(t + 1)
            kcopy(t + 1).start(priority=LO)
        vcopy(t).start(priority=LO)
    qproj(0)
    for xb in range(1, XS):
        xcopy(xb).wait()
    for t in range(1, XS):
        qproj(t)
    for xb in range(XS, B):
        xcopy(xb).wait()
    for t in range(XS, B):
        qproj(t)
    for g in range(1, (DQ - 1) // B + 1):
        wqcopy(g).wait()
    kcopy(0).wait()
    for t in range(B, DQ):
        qproj(t)
    qk(0, 0)
    weights_with_k(NBUF)
    kcopy(NBUF).start(priority=LO)

    t_light = T - DQ
    t_single = T - 2 - NSINGLE

    def heavy(i, c):
        t0 = i * 2
        waits(t0, 0, 2, True)
        step(t0, 0)
        step(t0 + 1, 1)
        refill(t0, 2)
        return c

    jax.lax.fori_loop(0, t_light // 2, heavy, 0)

    def light(i, c):
        t0 = t_light + i * 2
        fin(t0 - 2)
        fin(t0 - 3)
        waits(t0, 0, 2, False)
        step(t0, 0, do_qp=False)
        step(t0 + 1, 1, do_qp=False)
        refill(t0, 2)
        return c

    jax.lax.fori_loop(0, (t_single - t_light) // 2, light, 0)

    def single(i, c):
        t0 = t_single + i * 2
        for j in range(2):
            fin(t0 + j - 2)
            waits(t0 + j, j, 1, False)
            step(t0 + j, j, do_qp=False)
            refill(t0 + j, 1)
        return c

    assert t_single - 3 < T - B
    jax.lax.fori_loop(0, NSINGLE // 2, single, 0)

    t0 = T - 2
    fin(t0 - 2)
    waits(t0, 0, 2, False)
    for b in range(B - 3):
        ocopy(b).start(priority=HI)
    step(t0, 0, do_qp=False)
    finalize(B - 3, True)
    step(t0 + 1, 1, do_qk=False, do_qp=False)
    finalize(B - 2, True)
    outproj(T - 1, 1)
    finalize(B - 1, True)
    for b in range(B):
        ocopy(b).wait()


@jax.jit
def pallas_standalone__mha_block_cached__near_ridge_kernel(x, k_cache, v_cache, wq, wo):
    kt = jnp.swapaxes(k_cache, 2, 3).reshape(B, NG, PW, SK)
    vt = jnp.swapaxes(v_cache, 2, 3).reshape(B, NG, PW, SK)
    wo3 = wo.reshape(NG, PW, D)
    return pl.pallas_call(
        _kernel,
        in_specs=[pl.BlockSpec(memory_space=pl.ANY)] * 5,
        out_specs=pl.BlockSpec(memory_space=pl.ANY),
        out_shape=jax.ShapeDtypeStruct((B, SQ, D), BF16),
        scratch_shapes=[
            pltpu.VMEM((B, SQ, D), BF16),
            pltpu.VMEM((NG, D, PW), BF16),
            pltpu.VMEM((NG, PW, D), BF16),
            pltpu.VMEM((NBUF, PW, SK), BF16),
            pltpu.VMEM((NBUF, PW, SK), BF16),
            pltpu.VMEM((NQ, 2, SQ, 256), BF16),
            pltpu.VMEM((2, SQ, SK), F32), pltpu.VMEM((2, SQ, SK), F32),
            pltpu.VMEM((SQ, PW), BF16), pltpu.VMEM((SQ, PW), BF16),
            pltpu.VMEM((B, SQ, D), F32),
            pltpu.VMEM((B, SQ, D), BF16),
            pltpu.SemaphoreType.DMA((NBUF,)),
            pltpu.SemaphoreType.DMA((NBUF,)),
            pltpu.SemaphoreType.DMA((NG,)),
            pltpu.SemaphoreType.DMA((NG,)),
            pltpu.SemaphoreType.DMA((B,)),
            pltpu.SemaphoreType.DMA((B,)),
        ],
        compiler_params=pltpu.CompilerParams(
            vmem_limit_bytes=64 * 1024 * 1024,
            disable_bounds_checks=True,
            disable_semaphore_checks=True,
        ),
    )(x, wq, kt, vt, wo3)
```

```python
import jax
import jax.numpy as jnp
import jax.experimental.pallas as pl
import jax.experimental.pallas.tpu as pltpu

B, SQ, D = 8, 112, 640
H, SK, DH = 32, 512, 192
NG = H // 2
PW = 2 * DH
T = NG * B
NBUF = 8
DQ = 16
NQ = 16
NSINGLE = 8
XS = 4
HI, LO = 0, 1
SCALE = (DH ** -0.5) * 1.4426950408889634
NT = (((1,), (1,)), ((), ()))
F32 = jnp.float32
BF16 = jnp.bfloat16


def _kernel(x_hbm, wq_hbm, kt_hbm, vt_hbm, wo_hbm, out_hbm,
            xbuf, wqbuf, wobuf, kbuf, vbuf, qring,
            s0, s1, o0, o1, acc, obuf,
            ksem, vsem, wqsem, wosem, xsem, osem):
    ss = (s0, s1)
    oo = (o0, o1)

    def st(t):
        return isinstance(t, int)

    def grp(t):
        return t // B if st(t) else jax.lax.shift_right_logical(t, 3)

    def bat(t):
        return t % B if st(t) else jax.lax.bitwise_and(t, B - 1)

    def ring(t):
        return t % NBUF if st(t) else jax.lax.bitwise_and(t, NBUF - 1)

    def qslot(t):
        return t % NQ if st(t) else jax.lax.bitwise_and(t, NQ - 1)

    def when(cond, fn):
        if isinstance(cond, bool):
            if cond:
                fn()
        else:
            pl.when(cond)(fn)

    def land(a, b):
        if isinstance(a, bool) and isinstance(b, bool):
            return a and b
        return jnp.logical_and(a, b)

    def kcopy(t):
        sl = ring(t)
        return pltpu.make_async_copy(kt_hbm.at[bat(t), grp(t)], kbuf.at[sl], ksem.at[sl])

    def vcopy(t):
        sl = ring(t)
        return pltpu.make_async_copy(vt_hbm.at[bat(t), grp(t)], vbuf.at[sl], vsem.at[sl])

    def wqcopy(g):
        if st(g):
            src = wq_hbm.at[:, g * PW:(g + 1) * PW]
        else:
            src = wq_hbm.at[:, pl.ds(pl.multiple_of(g * PW, 128), PW)]
        return pltpu.make_async_copy(src, wqbuf.at[g], wqsem.at[g])

    def wocopy(g):
        return pltpu.make_async_copy(wo_hbm.at[g], wobuf.at[g], wosem.at[g])

    def xcopy(b):
        return pltpu.make_async_copy(x_hbm.at[b], xbuf.at[b], xsem.at[b])

    def ocopy(b):
        return pltpu.make_async_copy(obuf.at[b], out_hbm.at[b], osem.at[b])

    def arrival(buf, sem, idx):
        return pltpu.make_async_copy(buf.at[idx], buf.at[idx], sem.at[idx])

    lane = jax.lax.broadcasted_iota(jnp.int32, (SQ, 256), 1)

    def qproj(t):
        q = jnp.dot(xbuf[bat(t)], wqbuf[grp(t)], preferred_element_type=F32) * SCALE
        sl = qslot(t)
        qring[sl, 0] = jnp.where(lane < DH, q[:, 0:256], 0.0).astype(BF16)
        qring[sl, 1] = jnp.where(lane >= 64, q[:, 128:384], 0.0).astype(BF16)

    def qk(t, sl):
        ks = ring(t)
        qs = qslot(t)
        ss[sl][0] = jnp.dot(qring[qs, 0], kbuf[ks, 0:256, :], preferred_element_type=F32)
        ss[sl][1] = jnp.dot(qring[qs, 1], kbuf[ks, 128:384, :], preferred_element_type=F32)

    def softmax(sl):
        res = []
        for h in range(2):
            s = ss[sl][h]
            m = jnp.max(s, axis=-1, keepdims=True)
            p = jnp.exp2(s - m)
            l = jnp.sum(p, axis=-1, keepdims=True)
            res.append((p.astype(BF16), 1.0 / l))
        return res

    def pv(t, sl, res):
        vs = ring(t)
        (p0, r0), (p1, r1) = res
        ot0 = jax.lax.dot_general(vbuf[vs, 0:DH, :], p0, NT, preferred_element_type=F32)
        ot1 = jax.lax.dot_general(vbuf[vs, DH:PW, :], p1, NT, preferred_element_type=F32)
        o = jnp.concatenate([ot0, ot1], axis=0).T
        col = jax.lax.broadcasted_iota(jnp.int32, (SQ, PW), 1)
        oo[sl][...] = (o * jnp.where(col < DH, r0, r1)).astype(BF16)

    def outproj(t, sl, emit=False):
        b = bat(t)
        r = acc[b] + jnp.dot(oo[sl][...], wobuf[grp(t)], preferred_element_type=F32)
        if emit:
            obuf[b] = r.astype(BF16)
        if not (emit and st(t)):
            acc[b] = r

    def step(t, sl, do_qk=True, do_qp=True, emit=False):
        res = softmax(sl)
        if do_qk:
            qk(t + 1, 1 - sl)
        if do_qp:
            qproj(t + DQ)
        pv(t, sl, res)
        outproj(max(t - 1, 0) if st(t) else jnp.maximum(t - 1, 0), 1 - sl, emit)

    def weights_with_k(tk):
        tq = tk + DQ
        when(land(bat(tq) == 0, tq < T), lambda: wqcopy(grp(tq)).start(priority=HI))
        to = tk - 1
        when(bat(to) == 0, lambda: wocopy(grp(to)).start(priority=HI))

    def waits(t0, par, u, with_qp):
        todo = []

        def add(cond, buf, sem, idx):
            if cond is not False:
                todo.append((cond, arrival(buf, sem, idx)))
        for j in range(u):
            t = t0 + j
            add(not (st(t) and t + 1 >= T), kbuf, ksem, ring(t + 1))
            add(True, vbuf, vsem, ring(t))
        for j in range(u):
            t = t0 + j
            if with_qp and (par + j + DQ) % 2 == 0:
                add(bat(t + DQ) == 0, wqbuf, wqsem, grp(t + DQ))
            if (par + j) % 2 == 1:
                add(bat(t - 1) == 0, wobuf, wosem, grp(t - 1))
        for c, cp in todo:
            when(c, cp.wait)

    def refill(t0, u):
        for j in range(u):
            tk = t0 + 1 + j + NBUF
            tv = t0 + j + NBUF

            def issue_k():
                weights_with_k(tk)
                kcopy(tk).start(priority=LO)
            when(tk < T, issue_k)
            when(tv < T, lambda: vcopy(tv).start(priority=LO))

    xcopy(0).start(priority=HI)
    wqcopy(0).start(priority=HI)
    for xb in range(1, B):
        xcopy(xb).start(priority=HI)
    kcopy(0).start(priority=LO)
    acc[...] = jnp.zeros_like(acc)
    o1[...] = jnp.zeros_like(o1)
    xcopy(0).wait()
    wqcopy(0).wait()
    for g in range(1, DQ // B + 1):
        wqcopy(g).start(priority=HI)
    for t in range(NBUF):
        if t + 1 < NBUF:
            weights_with_k(t + 1)
            kcopy(t + 1).start(priority=LO)
        vcopy(t).start(priority=LO)
    qproj(0)
    for xb in range(1, XS):
        xcopy(xb).wait()
    for t in range(1, XS):
        qproj(t)
    for xb in range(XS, B):
        xcopy(xb).wait()
    for t in range(XS, B):
        qproj(t)
    for g in range(1, (DQ - 1) // B + 1):
        wqcopy(g).wait()
    kcopy(0).wait()
    for t in range(B, DQ):
        qproj(t)
    qk(0, 0)
    weights_with_k(NBUF)
    kcopy(NBUF).start(priority=LO)

    t_light = T - DQ
    t_single = T - 2 - NSINGLE

    def heavy(i, c):
        t0 = i * 2
        waits(t0, 0, 2, True)
        step(t0, 0)
        step(t0 + 1, 1)
        refill(t0, 2)
        return c

    jax.lax.fori_loop(0, t_light // 2, heavy, 0)

    def light(i, c):
        t0 = t_light + i * 2
        waits(t0, 0, 2, False)
        step(t0, 0, do_qp=False)
        step(t0 + 1, 1, do_qp=False)
        refill(t0, 2)
        return c

    assert t_single <= T - B + 1
    jax.lax.fori_loop(0, (t_single - t_light) // 2, light, 0)

    def single(i, c):
        t0 = t_single + i * 2
        for j in range(2):
            waits(t0 + j, j, 1, False)
            step(t0 + j, j, do_qp=False, emit=True)
            refill(t0 + j, 1)
        return c

    jax.lax.fori_loop(0, NSINGLE // 2, single, 0)

    t0 = T - 2
    waits(t0, 0, 2, False)
    for b in range(B - 3):
        ocopy(b).start(priority=HI)
    step(t0, 0, do_qp=False, emit=True)
    ocopy(B - 3).start(priority=HI)
    step(t0 + 1, 1, do_qk=False, do_qp=False, emit=True)
    ocopy(B - 2).start(priority=HI)
    outproj(T - 1, 1, True)
    ocopy(B - 1).start(priority=HI)
    for b in range(B):
        ocopy(b).wait()


@jax.jit
def pallas_standalone__mha_block_cached__near_ridge_kernel(x, k_cache, v_cache, wq, wo):
    kt = jnp.swapaxes(k_cache, 2, 3).reshape(B, NG, PW, SK)
    vt = jnp.swapaxes(v_cache, 2, 3).reshape(B, NG, PW, SK)
    wo3 = wo.reshape(NG, PW, D)
    return pl.pallas_call(
        _kernel,
        in_specs=[pl.BlockSpec(memory_space=pl.ANY)] * 5,
        out_specs=pl.BlockSpec(memory_space=pl.ANY),
        out_shape=jax.ShapeDtypeStruct((B, SQ, D), BF16),
        scratch_shapes=[
            pltpu.VMEM((B, SQ, D), BF16),
            pltpu.VMEM((NG, D, PW), BF16),
            pltpu.VMEM((NG, PW, D), BF16),
            pltpu.VMEM((NBUF, PW, SK), BF16),
            pltpu.VMEM((NBUF, PW, SK), BF16),
            pltpu.VMEM((NQ, 2, SQ, 256), BF16),
            pltpu.VMEM((2, SQ, SK), F32), pltpu.VMEM((2, SQ, SK), F32),
            pltpu.VMEM((SQ, PW), BF16), pltpu.VMEM((SQ, PW), BF16),
            pltpu.VMEM((B, SQ, D), F32),
            pltpu.VMEM((B, SQ, D), BF16),
            pltpu.SemaphoreType.DMA((NBUF,)),
            pltpu.SemaphoreType.DMA((NBUF,)),
            pltpu.SemaphoreType.DMA((NG,)),
            pltpu.SemaphoreType.DMA((NG,)),
            pltpu.SemaphoreType.DMA((B,)),
            pltpu.SemaphoreType.DMA((B,)),
        ],
        compiler_params=pltpu.CompilerParams(
            vmem_limit_bytes=64 * 1024 * 1024,
            disable_bounds_checks=True,
            disable_semaphore_checks=True,
        ),
    )(x, wq, kt, vt, wo3)
```

```python
import jax
import jax.numpy as jnp
import jax.experimental.pallas as pl
import jax.experimental.pallas.tpu as pltpu

B, SQ, D = 8, 112, 640
H, SK, DH = 32, 512, 192
NG = H // 2
PW = 2 * DH
T = NG * B
NBUF = 8
DQ = 16
NQ = 16
NSINGLE = 8
XS = 4
R0 = 8
HI, LO = 0, 1
SCALE = (DH ** -0.5) * 1.4426950408889634
NT = (((1,), (1,)), ((), ()))
F32 = jnp.float32
BF16 = jnp.bfloat16


def _kernel(x_hbm, wq_hbm, kt_hbm, vt_hbm, wo_hbm, out_hbm,
            xbuf, wqbuf, wobuf, kbuf, vbuf, qring,
            s0, s1, o0, o1, acc, obuf,
            ksem, vsem, wqsem, wosem, xsem, osem):
    ss = (s0, s1)
    oo = (o0, o1)

    def st(t):
        return isinstance(t, int)

    def grp(t):
        return t // B if st(t) else jax.lax.shift_right_logical(t, 3)

    def bat(t):
        return t % B if st(t) else jax.lax.bitwise_and(t, B - 1)

    def ring(t):
        return t % NBUF if st(t) else jax.lax.bitwise_and(t, NBUF - 1)

    def qslot(t):
        return t % NQ if st(t) else jax.lax.bitwise_and(t, NQ - 1)

    def when(cond, fn):
        if isinstance(cond, bool):
            if cond:
                fn()
        else:
            pl.when(cond)(fn)

    def land(a, b):
        if isinstance(a, bool) and isinstance(b, bool):
            return a and b
        return jnp.logical_and(a, b)

    def kv_start(hbm, buf, sem, t):
        sl = ring(t)
        src = hbm.at[bat(t), grp(t)]
        dst = buf.at[sl]
        if R0:
            pltpu.make_async_copy(src.at[0:R0], dst.at[0:R0], sem.at[sl]).start(priority=HI)
        pltpu.make_async_copy(src.at[R0:PW], dst.at[R0:PW], sem.at[sl]).start(priority=LO)

    def kstart(t):
        kv_start(kt_hbm, kbuf, ksem, t)

    def vstart(t):
        kv_start(vt_hbm, vbuf, vsem, t)

    def wqcopy(g):
        if st(g):
            src = wq_hbm.at[:, g * PW:(g + 1) * PW]
        else:
            src = wq_hbm.at[:, pl.ds(pl.multiple_of(g * PW, 128), PW)]
        return pltpu.make_async_copy(src, wqbuf.at[g], wqsem.at[g])

    def wocopy(g):
        return pltpu.make_async_copy(wo_hbm.at[g], wobuf.at[g], wosem.at[g])

    def xcopy(b):
        return pltpu.make_async_copy(x_hbm.at[b], xbuf.at[b], xsem.at[b])

    def ocopy(b):
        return pltpu.make_async_copy(obuf.at[b], out_hbm.at[b], osem.at[b])

    def arrival(buf, sem, idx):
        return pltpu.make_async_copy(buf.at[idx], buf.at[idx], sem.at[idx])

    lane = jax.lax.broadcasted_iota(jnp.int32, (SQ, 256), 1)

    def qproj(t):
        q = jnp.dot(xbuf[bat(t)], wqbuf[grp(t)], preferred_element_type=F32) * SCALE
        sl = qslot(t)
        qring[sl, 0] = jnp.where(lane < DH, q[:, 0:256], 0.0).astype(BF16)
        qring[sl, 1] = jnp.where(lane >= 64, q[:, 128:384], 0.0).astype(BF16)

    def qk(t, sl):
        ks = ring(t)
        qs = qslot(t)
        ss[sl][0] = jnp.dot(qring[qs, 0], kbuf[ks, 0:256, :], preferred_element_type=F32)
        ss[sl][1] = jnp.dot(qring[qs, 1], kbuf[ks, 128:384, :], preferred_element_type=F32)

    def softmax(sl):
        res = []
        for h in range(2):
            s = ss[sl][h]
            m = jnp.max(s, axis=-1, keepdims=True)
            p = jnp.exp2(s - m)
            l = jnp.sum(p, axis=-1, keepdims=True)
            res.append((p.astype(BF16), 1.0 / l))
        return res

    def pv(t, sl, res):
        vs = ring(t)
        (p0, r0), (p1, r1) = res
        ot0 = jax.lax.dot_general(vbuf[vs, 0:DH, :], p0, NT, preferred_element_type=F32)
        ot1 = jax.lax.dot_general(vbuf[vs, DH:PW, :], p1, NT, preferred_element_type=F32)
        o = jnp.concatenate([ot0, ot1], axis=0).T
        col = jax.lax.broadcasted_iota(jnp.int32, (SQ, PW), 1)
        oo[sl][...] = (o * jnp.where(col < DH, r0, r1)).astype(BF16)

    def outproj(t, sl, emit=False):
        b = bat(t)
        r = acc[b] + jnp.dot(oo[sl][...], wobuf[grp(t)], preferred_element_type=F32)
        if emit:
            obuf[b] = r.astype(BF16)
        if not (emit and st(t)):
            acc[b] = r

    def step(t, sl, do_qk=True, do_qp=True, emit=False):
        res = softmax(sl)
        if do_qk:
            qk(t + 1, 1 - sl)
        if do_qp:
            qproj(t + DQ)
        pv(t, sl, res)
        outproj(max(t - 1, 0) if st(t) else jnp.maximum(t - 1, 0), 1 - sl, emit)

    def weights_with_k(tk):
        tq = tk + DQ
        when(land(bat(tq) == 0, tq < T), lambda: wqcopy(grp(tq)).start(priority=HI))
        to = tk - 1
        when(bat(to) == 0, lambda: wocopy(grp(to)).start(priority=HI))

    def waits(t0, par, u, with_qp):
        todo = []

        def add(cond, buf, sem, idx):
            if cond is not False:
                todo.append((cond, arrival(buf, sem, idx)))
        for j in range(u):
            t = t0 + j
            add(not (st(t) and t + 1 >= T), kbuf, ksem, ring(t + 1))
            add(True, vbuf, vsem, ring(t))
        for j in range(u):
            t = t0 + j
            if with_qp and (par + j + DQ) % 2 == 0:
                add(bat(t + DQ) == 0, wqbuf, wqsem, grp(t + DQ))
            if (par + j) % 2 == 1:
                add(bat(t - 1) == 0, wobuf, wosem, grp(t - 1))
        for c, cp in todo:
            when(c, cp.wait)

    def refill(t0, u):
        for j in range(u):
            tk = t0 + 1 + j + NBUF
            tv = t0 + j + NBUF

            def issue_k():
                weights_with_k(tk)
                kstart(tk)
            when(tk < T, issue_k)
            when(tv < T, lambda: vstart(tv))

    xcopy(0).start(priority=HI)
    wqcopy(0).start(priority=HI)
    for xb in range(1, B):
        xcopy(xb).start(priority=HI)
    kstart(0)
    acc[...] = jnp.zeros_like(acc)
    o1[...] = jnp.zeros_like(o1)
    xcopy(0).wait()
    wqcopy(0).wait()
    for g in range(1, DQ // B + 1):
        wqcopy(g).start(priority=HI)
    for t in range(NBUF):
        if t + 1 < NBUF:
            weights_with_k(t + 1)
            kstart(t + 1)
        vstart(t)
    qproj(0)
    for xb in range(1, XS):
        xcopy(xb).wait()
    for t in range(1, XS):
        qproj(t)
    for xb in range(XS, B):
        xcopy(xb).wait()
    for t in range(XS, B):
        qproj(t)
    for g in range(1, (DQ - 1) // B + 1):
        wqcopy(g).wait()
    arrival(kbuf, ksem, 0).wait()
    for t in range(B, DQ):
        qproj(t)
    qk(0, 0)
    weights_with_k(NBUF)
    kstart(NBUF)

    t_light = T - DQ
    t_single = T - 2 - NSINGLE

    def heavy(i, c):
        t0 = i * 2
        waits(t0, 0, 2, True)
        step(t0, 0)
        step(t0 + 1, 1)
        refill(t0, 2)
        return c

    jax.lax.fori_loop(0, t_light // 2, heavy, 0)

    def light(i, c):
        t0 = t_light + i * 2
        waits(t0, 0, 2, False)
        step(t0, 0, do_qp=False)
        step(t0 + 1, 1, do_qp=False)
        refill(t0, 2)
        return c

    assert t_single <= T - B + 1
    jax.lax.fori_loop(0, (t_single - t_light) // 2, light, 0)

    def single(i, c):
        t0 = t_single + i * 2
        for j in range(2):
            waits(t0 + j, j, 1, False)
            step(t0 + j, j, do_qp=False, emit=True)
            refill(t0 + j, 1)
        return c

    jax.lax.fori_loop(0, NSINGLE // 2, single, 0)

    t0 = T - 2
    waits(t0, 0, 2, False)
    for b in range(B - 3):
        ocopy(b).start(priority=HI)
    step(t0, 0, do_qp=False, emit=True)
    ocopy(B - 3).start(priority=HI)
    step(t0 + 1, 1, do_qk=False, do_qp=False, emit=True)
    ocopy(B - 2).start(priority=HI)
    outproj(T - 1, 1, True)
    ocopy(B - 1).start(priority=HI)
    for b in range(B):
        ocopy(b).wait()


@jax.jit
def pallas_standalone__mha_block_cached__near_ridge_kernel(x, k_cache, v_cache, wq, wo):
    kt = jnp.swapaxes(k_cache, 2, 3).reshape(B, NG, PW, SK)
    vt = jnp.swapaxes(v_cache, 2, 3).reshape(B, NG, PW, SK)
    wo3 = wo.reshape(NG, PW, D)
    return pl.pallas_call(
        _kernel,
        in_specs=[pl.BlockSpec(memory_space=pl.ANY)] * 5,
        out_specs=pl.BlockSpec(memory_space=pl.ANY),
        out_shape=jax.ShapeDtypeStruct((B, SQ, D), BF16),
        scratch_shapes=[
            pltpu.VMEM((B, SQ, D), BF16),
            pltpu.VMEM((NG, D, PW), BF16),
            pltpu.VMEM((NG, PW, D), BF16),
            pltpu.VMEM((NBUF, PW, SK), BF16),
            pltpu.VMEM((NBUF, PW, SK), BF16),
            pltpu.VMEM((NQ, 2, SQ, 256), BF16),
            pltpu.VMEM((2, SQ, SK), F32), pltpu.VMEM((2, SQ, SK), F32),
            pltpu.VMEM((SQ, PW), BF16), pltpu.VMEM((SQ, PW), BF16),
            pltpu.VMEM((B, SQ, D), F32),
            pltpu.VMEM((B, SQ, D), BF16),
            pltpu.SemaphoreType.DMA((NBUF,)),
            pltpu.SemaphoreType.DMA((NBUF,)),
            pltpu.SemaphoreType.DMA((NG,)),
            pltpu.SemaphoreType.DMA((NG,)),
            pltpu.SemaphoreType.DMA((B,)),
            pltpu.SemaphoreType.DMA((B,)),
        ],
        compiler_params=pltpu.CompilerParams(
            vmem_limit_bytes=64 * 1024 * 1024,
            disable_bounds_checks=True,
            disable_semaphore_checks=True,
        ),
    )(x, wq, kt, vt, wo3)
```

```python
import jax
import jax.numpy as jnp
import jax.experimental.pallas as pl
import jax.experimental.pallas.tpu as pltpu

B, SQ, D = 8, 112, 640
H, SK, DH = 32, 512, 192
NG = H // 2
PW = 2 * DH
T = NG * B
NBUF = 8
DQ = 2 * B
NQ = 16
NSINGLE = 6
XS = 4
R0 = 8
WQR, WOR = D // B, PW // B
WQ_LEAD, WO_LEAD = 6, 5
HI, LO = 0, 1
SCALE = (DH ** -0.5) * 1.4426950408889634
NT = (((1,), (1,)), ((), ()))
F32 = jnp.float32
BF16 = jnp.bfloat16


def _kernel(x_hbm, wq_hbm, kt_hbm, vt_hbm, wo_hbm, out_hbm,
            xbuf, wqbuf, wobuf, kbuf, vbuf, qring,
            s0, s1, o0, o1, acc, obuf,
            ksem, vsem, wqsem, wosem, xsem, osem):
    ss = (s0, s1)
    oo = (o0, o1)

    def st(t):
        return isinstance(t, int)

    def grp(t):
        return t // B if st(t) else jax.lax.shift_right_logical(t, 3)

    def bat(t):
        return t % B if st(t) else jax.lax.bitwise_and(t, B - 1)

    def ring(t):
        return t % NBUF if st(t) else jax.lax.bitwise_and(t, NBUF - 1)

    def qslot(t):
        return t % NQ if st(t) else jax.lax.bitwise_and(t, NQ - 1)

    def when(cond, fn):
        if isinstance(cond, bool):
            if cond:
                fn()
        else:
            pl.when(cond)(fn)

    def land(a, b):
        if isinstance(a, bool) and isinstance(b, bool):
            return a and b
        return jnp.logical_and(a, b)

    def kv_start(hbm, buf, sem, t):
        sl = ring(t)
        src = hbm.at[bat(t), grp(t)]
        dst = buf.at[sl]
        pltpu.make_async_copy(src.at[0:R0], dst.at[0:R0], sem.at[sl]).start(priority=HI)
        pltpu.make_async_copy(src.at[R0:PW], dst.at[R0:PW], sem.at[sl]).start(priority=LO)

    def kstart(t):
        kv_start(kt_hbm, kbuf, ksem, t)

    def vstart(t):
        kv_start(vt_hbm, vbuf, vsem, t)

    def wqcopy(g):
        return pltpu.make_async_copy(wq_hbm.at[:, g * PW:(g + 1) * PW], wqbuf.at[g], wqsem.at[g])

    def wocopy(g):
        return pltpu.make_async_copy(wo_hbm.at[g], wobuf.at[g], wosem.at[g])

    def wq_piece(g, i):
        rows = pl.ds(i * WQR, WQR) if st(i) else pl.ds(pl.multiple_of(i * WQR, 16), WQR)
        cols = pl.ds(g * PW, PW) if st(g) else pl.ds(pl.multiple_of(g * PW, 128), PW)
        return pltpu.make_async_copy(wq_hbm.at[rows, cols], wqbuf.at[g, rows], wqsem.at[g])

    def wo_piece(g, i):
        rows = pl.ds(i * WOR, WOR) if st(i) else pl.ds(pl.multiple_of(i * WOR, 16), WOR)
        return pltpu.make_async_copy(wo_hbm.at[g, rows], wobuf.at[g, rows], wosem.at[g])

    def xcopy(b):
        return pltpu.make_async_copy(x_hbm.at[b], xbuf.at[b], xsem.at[b])

    def ocopy(b):
        return pltpu.make_async_copy(obuf.at[b], out_hbm.at[b], osem.at[b])

    def arrival(buf, sem, idx):
        return pltpu.make_async_copy(buf.at[idx], buf.at[idx], sem.at[idx])

    lane = jax.lax.broadcasted_iota(jnp.int32, (SQ, 256), 1)

    def qproj(t):
        q = jnp.dot(xbuf[bat(t)], wqbuf[grp(t)], preferred_element_type=F32) * SCALE
        sl = qslot(t)
        qring[sl, 0] = jnp.where(lane < DH, q[:, 0:256], 0.0).astype(BF16)
        qring[sl, 1] = jnp.where(lane >= 64, q[:, 128:384], 0.0).astype(BF16)

    def qk(t, sl):
        ks = ring(t)
        qs = qslot(t)
        ss[sl][0] = jnp.dot(qring[qs, 0], kbuf[ks, 0:256, :], preferred_element_type=F32)
        ss[sl][1] = jnp.dot(qring[qs, 1], kbuf[ks, 128:384, :], preferred_element_type=F32)

    def softmax(sl):
        res = []
        for h in range(2):
            s = ss[sl][h]
            m = jnp.max(s, axis=-1, keepdims=True)
            p = jnp.exp2(s - m)
            l = jnp.sum(p, axis=-1, keepdims=True)
            res.append((p.astype(BF16), 1.0 / l))
        return res

    def pv(t, sl, res):
        vs = ring(t)
        (p0, r0), (p1, r1) = res
        ot0 = jax.lax.dot_general(vbuf[vs, 0:DH, :], p0, NT, preferred_element_type=F32)
        ot1 = jax.lax.dot_general(vbuf[vs, DH:PW, :], p1, NT, preferred_element_type=F32)
        o = jnp.concatenate([ot0, ot1], axis=0).T
        col = jax.lax.broadcasted_iota(jnp.int32, (SQ, PW), 1)
        oo[sl][...] = (o * jnp.where(col < DH, r0, r1)).astype(BF16)

    def outproj(t, sl, emit=False):
        b = bat(t)
        r = acc[b] + jnp.dot(oo[sl][...], wobuf[grp(t)], preferred_element_type=F32)
        if emit:
            obuf[b] = r.astype(BF16)
        if not (emit and st(t)):
            acc[b] = r

    def step(t, sl, do_qk=True, do_qp=True, emit=False):
        res = softmax(sl)
        if do_qk:
            qk(t + 1, 1 - sl)
        if do_qp:
            qproj(t + DQ)
        pv(t, sl, res)
        outproj(max(t - 1, 0) if st(t) else jnp.maximum(t - 1, 0), 1 - sl, emit)

    first_wq = B * (DQ // B + 1)
    assert 1 + DQ + WQ_LEAD <= first_wq and 1 + WO_LEAD <= B

    def issue(tk, tv):
        when(tk < T, lambda: kstart(tk))
        uq = tk + DQ + WQ_LEAD
        when(land(uq >= first_wq, uq < T), lambda: wq_piece(grp(uq), bat(uq)).start(priority=HI))
        when(tv < T, lambda: vstart(tv))
        uo = tk + WO_LEAD
        when(land(uo >= B, uo < T), lambda: wo_piece(grp(uo), bat(uo)).start(priority=HI))

    def refill(t):
        issue(t + 1 + NBUF, t + NBUF)

    def waits(t0, par, u, with_qp):
        todo = []

        def add(cond, buf, sem, idx):
            if cond is not False:
                todo.append((cond, arrival(buf, sem, idx)))
        for j in range(u):
            t = t0 + j
            add(not (st(t) and t + 1 >= T), kbuf, ksem, ring(t + 1))
            add(True, vbuf, vsem, ring(t))
        for j in range(u):
            t = t0 + j
            if with_qp and (par + j + DQ) % 2 == 0:
                add(bat(t + DQ) == 0, wqbuf, wqsem, grp(t + DQ))
            if (par + j) % 2 == 1:
                add(bat(t - 1) == 0, wobuf, wosem, grp(t - 1))
        for c, cp in todo:
            when(c, cp.wait)

    xcopy(0).start(priority=HI)
    wqcopy(0).start(priority=HI)
    for xb in range(1, B):
        xcopy(xb).start(priority=LO)
    kstart(0)
    acc[...] = jnp.zeros_like(acc)
    o1[...] = jnp.zeros_like(o1)
    xcopy(0).wait()
    wqcopy(0).wait()
    for t in range(NBUF - 1):
        issue(t + 1, t)
    qproj(0)
    for xb in range(1, XS):
        xcopy(xb).wait()
    for t in range(1, XS):
        qproj(t)
    for xb in range(XS, B):
        xcopy(xb).wait()
    wqcopy(1).start(priority=HI)
    for t in range(XS, B):
        qproj(t)
    wqcopy(1).wait()
    arrival(kbuf, ksem, 0).wait()
    wqcopy(2).start(priority=HI)
    wocopy(0).start(priority=HI)
    for t in range(B, DQ):
        qproj(t)
    qk(0, 0)
    issue(NBUF, NBUF - 1)

    t_light = T - DQ
    t_single = T - 2 - NSINGLE

    def heavy(i, c):
        t0 = i * 2
        waits(t0, 0, 2, True)
        step(t0, 0)
        step(t0 + 1, 1)
        refill(t0)
        refill(t0 + 1)
        return c

    jax.lax.fori_loop(0, t_light // 2, heavy, 0)

    def light(i, c):
        t0 = t_light + i * 2
        waits(t0, 0, 2, False)
        step(t0, 0, do_qp=False)
        step(t0 + 1, 1, do_qp=False)
        refill(t0)
        refill(t0 + 1)
        return c

    assert t_single <= T - B + 1
    jax.lax.fori_loop(0, (t_single - t_light) // 2, light, 0)

    def single(i, c):
        t0 = t_single + i * 2
        for j in range(2):
            waits(t0 + j, j, 1, False)
            step(t0 + j, j, do_qp=False, emit=True)
            refill(t0 + j)
        return c

    jax.lax.fori_loop(0, NSINGLE // 2, single, 0)

    t0 = T - 2
    waits(t0, 0, 2, False)
    for b in range(B - 3):
        ocopy(b).start(priority=HI)
    step(t0, 0, do_qp=False, emit=True)
    ocopy(B - 3).start(priority=HI)
    step(t0 + 1, 1, do_qk=False, do_qp=False, emit=True)
    ocopy(B - 2).start(priority=HI)
    outproj(T - 1, 1, True)
    ocopy(B - 1).start(priority=HI)
    for b in range(B):
        ocopy(b).wait()


@jax.jit
def pallas_standalone__mha_block_cached__near_ridge_kernel(x, k_cache, v_cache, wq, wo):
    kt = jnp.swapaxes(k_cache, 2, 3).reshape(B, NG, PW, SK)
    vt = jnp.swapaxes(v_cache, 2, 3).reshape(B, NG, PW, SK)
    wo3 = wo.reshape(NG, PW, D)
    return pl.pallas_call(
        _kernel,
        in_specs=[pl.BlockSpec(memory_space=pl.ANY)] * 5,
        out_specs=pl.BlockSpec(memory_space=pl.ANY),
        out_shape=jax.ShapeDtypeStruct((B, SQ, D), BF16),
        scratch_shapes=[
            pltpu.VMEM((B, SQ, D), BF16),
            pltpu.VMEM((NG, D, PW), BF16),
            pltpu.VMEM((NG, PW, D), BF16),
            pltpu.VMEM((NBUF, PW, SK), BF16),
            pltpu.VMEM((NBUF, PW, SK), BF16),
            pltpu.VMEM((NQ, 2, SQ, 256), BF16),
            pltpu.VMEM((2, SQ, SK), F32), pltpu.VMEM((2, SQ, SK), F32),
            pltpu.VMEM((SQ, PW), BF16), pltpu.VMEM((SQ, PW), BF16),
            pltpu.VMEM((B, SQ, D), F32),
            pltpu.VMEM((B, SQ, D), BF16),
            pltpu.SemaphoreType.DMA((NBUF,)),
            pltpu.SemaphoreType.DMA((NBUF,)),
            pltpu.SemaphoreType.DMA((NG,)),
            pltpu.SemaphoreType.DMA((NG,)),
            pltpu.SemaphoreType.DMA((B,)),
            pltpu.SemaphoreType.DMA((B,)),
        ],
        compiler_params=pltpu.CompilerParams(
            vmem_limit_bytes=64 * 1024 * 1024,
            disable_bounds_checks=True,
            disable_semaphore_checks=True,
        ),
    )(x, wq, kt, vt, wo3)
```

```python
import jax
import jax.numpy as jnp
import jax.experimental.pallas as pl
import jax.experimental.pallas.tpu as pltpu

B, SQ, D = 8, 112, 640
H, SK, DH = 32, 512, 192
NG = H // 2
PW = 2 * DH
T = NG * B
NBUF = 8
PD = 7
UH, UL = 4, 2
NSINGLE = 2
DQ = 3 * B
NQ = 32
XS = 4
NSEG, R0 = 2, 8
WQR, WOR = D // B, PW // B
WQ_LEAD, WO_LEAD = 6, 5
HI, LO = 0, 1
SCALE = (DH ** -0.5) * 1.4426950408889634
NT = (((1,), (1,)), ((), ()))
F32 = jnp.float32
BF16 = jnp.bfloat16


def _kernel(x_hbm, wq_hbm, kt_hbm, vt_hbm, wo_hbm, out_hbm,
            xbuf, wqbuf, wobuf, kbuf, vbuf, qring,
            s0, s1, o0, o1, acc, obuf,
            ksem, vsem, wqsem, wosem, xsem, osem):
    ss = (s0, s1)
    oo = (o0, o1)

    def st(t):
        return isinstance(t, int)

    def grp(t):
        return t // B if st(t) else jax.lax.shift_right_logical(t, 3)

    def bat(t):
        return t % B if st(t) else jax.lax.bitwise_and(t, B - 1)

    def ring(t):
        return t % NBUF if st(t) else jax.lax.bitwise_and(t, NBUF - 1)

    def qslot(t):
        return t % NQ if st(t) else jax.lax.bitwise_and(t, NQ - 1)

    def when(cond, fn):
        if isinstance(cond, bool):
            if cond:
                fn()
        else:
            pl.when(cond)(fn)

    def land(a, b):
        if isinstance(a, bool) and isinstance(b, bool):
            return a and b
        return jnp.logical_and(a, b)

    def kv_start(hbm, buf, sem, t):
        sl = ring(t)
        src = hbm.at[bat(t), grp(t)]
        dst = buf.at[sl]
        seg = PW // NSEG
        for i in range(NSEG):
            lo = i * seg
            pltpu.make_async_copy(src.at[lo:lo + R0], dst.at[lo:lo + R0], sem.at[sl]).start(priority=HI)
            pltpu.make_async_copy(src.at[lo + R0:lo + seg], dst.at[lo + R0:lo + seg], sem.at[sl]).start(priority=LO)

    def kstart(t):
        kv_start(kt_hbm, kbuf, ksem, t)

    def vstart(t):
        kv_start(vt_hbm, vbuf, vsem, t)

    def wqcopy(g):
        return pltpu.make_async_copy(wq_hbm.at[:, g * PW:(g + 1) * PW], wqbuf.at[g], wqsem.at[g])

    def wocopy(g):
        return pltpu.make_async_copy(wo_hbm.at[g], wobuf.at[g], wosem.at[g])

    def wq_piece(g, i):
        rows = pl.ds(i * WQR, WQR) if st(i) else pl.ds(pl.multiple_of(i * WQR, 16), WQR)
        cols = pl.ds(g * PW, PW) if st(g) else pl.ds(pl.multiple_of(g * PW, 128), PW)
        return pltpu.make_async_copy(wq_hbm.at[rows, cols], wqbuf.at[g, rows], wqsem.at[g])

    def wo_piece(g, i):
        rows = pl.ds(i * WOR, WOR) if st(i) else pl.ds(pl.multiple_of(i * WOR, 16), WOR)
        return pltpu.make_async_copy(wo_hbm.at[g, rows], wobuf.at[g, rows], wosem.at[g])

    def xcopy(b):
        return pltpu.make_async_copy(x_hbm.at[b], xbuf.at[b], xsem.at[b])

    def ocopy(b):
        return pltpu.make_async_copy(obuf.at[b], out_hbm.at[b], osem.at[b])

    def arrival(buf, sem, idx):
        return pltpu.make_async_copy(buf.at[idx], buf.at[idx], sem.at[idx])

    lane = jax.lax.broadcasted_iota(jnp.int32, (SQ, 256), 1)

    def qproj(t):
        q = jnp.dot(xbuf[bat(t)], wqbuf[grp(t)], preferred_element_type=F32) * SCALE
        sl = qslot(t)
        qring[sl, 0] = jnp.where(lane < DH, q[:, 0:256], 0.0).astype(BF16)
        qring[sl, 1] = jnp.where(lane >= 64, q[:, 128:384], 0.0).astype(BF16)

    def qk(t, sl):
        ks = ring(t)
        qs = qslot(t)
        ss[sl][0] = jnp.dot(qring[qs, 0], kbuf[ks, 0:256, :], preferred_element_type=F32)
        ss[sl][1] = jnp.dot(qring[qs, 1], kbuf[ks, 128:384, :], preferred_element_type=F32)

    def softmax(sl):
        res = []
        for h in range(2):
            s = ss[sl][h]
            m = jnp.max(s, axis=-1, keepdims=True)
            p = jnp.exp2(s - m)
            l = jnp.sum(p, axis=-1, keepdims=True)
            res.append((p.astype(BF16), 1.0 / l))
        return res

    def pv(t, sl, res):
        vs = ring(t)
        (p0, r0), (p1, r1) = res
        ot0 = jax.lax.dot_general(vbuf[vs, 0:DH, :], p0, NT, preferred_element_type=F32)
        ot1 = jax.lax.dot_general(vbuf[vs, DH:PW, :], p1, NT, preferred_element_type=F32)
        o = jnp.concatenate([ot0, ot1], axis=0).T
        col = jax.lax.broadcasted_iota(jnp.int32, (SQ, PW), 1)
        oo[sl][...] = (o * jnp.where(col < DH, r0, r1)).astype(BF16)

    def outproj(t, sl, emit=False):
        b = bat(t)
        r = acc[b] + jnp.dot(oo[sl][...], wobuf[grp(t)], preferred_element_type=F32)
        if emit:
            obuf[b] = r.astype(BF16)
        if not (emit and st(t)):
            acc[b] = r

    def step(t, sl, do_qk=True, do_qp=True, emit=False):
        res = softmax(sl)
        if do_qk:
            qk(t + 1, 1 - sl)
        if do_qp:
            qproj(t + DQ)
        pv(t, sl, res)
        outproj(max(t - 1, 0) if st(t) else jnp.maximum(t - 1, 0), 1 - sl, emit)

    first_wq = B * (DQ // B + 1)
    assert 1 + DQ + WQ_LEAD <= first_wq and 1 + WO_LEAD <= B

    def issue(tk, tv):
        when(tk < T, lambda: kstart(tk))
        uq = tk + DQ + WQ_LEAD
        when(land(uq >= first_wq, uq < T), lambda: wq_piece(grp(uq), bat(uq)).start(priority=HI))
        when(tv < T, lambda: vstart(tv))
        uo = tk + WO_LEAD
        when(land(uo >= B, uo < T), lambda: wo_piece(grp(uo), bat(uo)).start(priority=HI))

    def refill(t):
        issue(t + 1 + PD, t + PD)

    def waits(t0, par, u, with_qp, align=2):
        todo = []

        def add(cond, buf, sem, idx):
            if cond is not False:
                todo.append((cond, arrival(buf, sem, idx)))
        for j in range(u):
            t = t0 + j
            add(not (st(t) and t + 1 >= T), kbuf, ksem, ring(t + 1))
            add(True, vbuf, vsem, ring(t))
        for j in range(u):
            t = t0 + j
            if with_qp and (par + j + DQ) % align == 0:
                add(bat(t + DQ) == 0, wqbuf, wqsem, grp(t + DQ))
            if (par + j - 1) % align == 0:
                add(bat(t - 1) == 0, wobuf, wosem, grp(t - 1))
        for c, cp in todo:
            when(c, cp.wait)

    xcopy(0).start(priority=HI)
    wqcopy(0).start(priority=HI)
    for xb in range(1, B):
        xcopy(xb).start(priority=LO)
    kstart(0)
    acc[...] = jnp.zeros_like(acc)
    o1[...] = jnp.zeros_like(o1)
    xcopy(0).wait()
    wqcopy(0).wait()
    issue(1, 0)
    qproj(0)
    for xb in range(1, XS):
        xcopy(xb).wait()
    for t in range(1, PD - 1):
        issue(t + 1, t)
    for t in range(1, XS):
        qproj(t)
    for xb in range(XS, B):
        xcopy(xb).wait()
    wqcopy(1).start(priority=HI)
    for t in range(XS, B):
        qproj(t)
    NGQ = DQ // B
    for g in range(1, NGQ):
        wqcopy(g).wait()
        if g == NGQ - 1:
            arrival(kbuf, ksem, 0).wait()
        wqcopy(g + 1).start(priority=HI)
        if g == 1:
            wocopy(0).start(priority=HI)
        for t in range(g * B, (g + 1) * B):
            qproj(t)
    qk(0, 0)
    issue(PD, PD - 1)

    t_light = T - DQ
    t_single = T - 2 - NSINGLE

    def run_block(t0, u, do_qp, emit=False):
        waits(t0, 0, u, do_qp, min(u, 8))
        for j in range(u):
            step(t0 + j, j % 2, do_qp=do_qp, emit=emit)
            refill(t0 + j)

    def heavy(i, c):
        run_block(i * UH, UH, True)
        return c

    assert t_light % UH == 0 and UH + 1 <= PD <= NBUF
    jax.lax.fori_loop(0, t_light // UH, heavy, 0)

    def light(i, c):
        run_block(t_light + i * UL, UL, False, True)
        return c

    assert (t_single - t_light) % UL == 0
    jax.lax.fori_loop(0, (t_single - t_light) // UL, light, 0)

    def single(i, c):
        t0 = t_single + i * 2
        for j in range(2):
            waits(t0 + j, j, 1, False)
            step(t0 + j, j, do_qp=False, emit=True)
            refill(t0 + j)
        return c

    jax.lax.fori_loop(0, NSINGLE // 2, single, 0)

    t0 = T - 2
    waits(t0, 0, 2, False)
    for b in range(B - 3):
        ocopy(b).start(priority=HI)
    step(t0, 0, do_qp=False, emit=True)
    ocopy(B - 3).start(priority=HI)
    step(t0 + 1, 1, do_qk=False, do_qp=False, emit=True)
    ocopy(B - 2).start(priority=HI)
    outproj(T - 1, 1, True)
    ocopy(B - 1).start(priority=HI)
    for b in range(B):
        ocopy(b).wait()


@jax.jit
def pallas_standalone__mha_block_cached__near_ridge_kernel(x, k_cache, v_cache, wq, wo):
    kt = jnp.swapaxes(k_cache, 2, 3).reshape(B, NG, PW, SK)
    vt = jnp.swapaxes(v_cache, 2, 3).reshape(B, NG, PW, SK)
    wo3 = wo.reshape(NG, PW, D)
    return pl.pallas_call(
        _kernel,
        in_specs=[pl.BlockSpec(memory_space=pl.ANY)] * 5,
        out_specs=pl.BlockSpec(memory_space=pl.ANY),
        out_shape=jax.ShapeDtypeStruct((B, SQ, D), BF16),
        scratch_shapes=[
            pltpu.VMEM((B, SQ, D), BF16),
            pltpu.VMEM((NG, D, PW), BF16),
            pltpu.VMEM((NG, PW, D), BF16),
            pltpu.VMEM((NBUF, PW, SK), BF16),
            pltpu.VMEM((NBUF, PW, SK), BF16),
            pltpu.VMEM((NQ, 2, SQ, 256), BF16),
            pltpu.VMEM((2, SQ, SK), F32), pltpu.VMEM((2, SQ, SK), F32),
            pltpu.VMEM((SQ, PW), BF16), pltpu.VMEM((SQ, PW), BF16),
            pltpu.VMEM((B, SQ, D), F32),
            pltpu.VMEM((B, SQ, D), BF16),
            pltpu.SemaphoreType.DMA((NBUF,)),
            pltpu.SemaphoreType.DMA((NBUF,)),
            pltpu.SemaphoreType.DMA((NG,)),
            pltpu.SemaphoreType.DMA((NG,)),
            pltpu.SemaphoreType.DMA((B,)),
            pltpu.SemaphoreType.DMA((B,)),
        ],
        compiler_params=pltpu.CompilerParams(
            vmem_limit_bytes=64 * 1024 * 1024,
            disable_bounds_checks=True,
            disable_semaphore_checks=True,
        ),
    )(x, wq, kt, vt, wo3)
```

```python
import jax
import jax.numpy as jnp
import jax.experimental.pallas as pl
import jax.experimental.pallas.tpu as pltpu

B, SQ, D = 8, 112, 640
H, SK, DH = 32, 512, 192
NG = H // 2
PW = 2 * DH
T = NG * B
NBUF = 8
PD = 7
UH, UL = 4, 2
DQ = 3 * B
NQ = 32
XS = 4
NSEG, R0 = 2, 8
WQR, WOR = D // B, PW // B
WQ_LEAD, WO_LEAD = 3, 2
HI, LO = 0, 1
SCALE = (DH ** -0.5) * 1.4426950408889634
NT = (((1,), (1,)), ((), ()))
F32 = jnp.float32
BF16 = jnp.bfloat16


def _kernel(x_hbm, wq_hbm, kt_hbm, vt_hbm, wo_hbm, out_hbm,
            xbuf, wqbuf, wobuf, kbuf, vbuf, qring,
            s0, s1, o0, o1, acc, obuf,
            ksem, vsem, wqsem, wosem, xsem, osem):
    ss = (s0, s1)
    oo = (o0, o1)

    def st(t):
        return isinstance(t, int)

    def grp(t):
        return t // B if st(t) else jax.lax.shift_right_logical(t, 3)

    def bat(t):
        return t % B if st(t) else jax.lax.bitwise_and(t, B - 1)

    def ring(t):
        return t % NBUF if st(t) else jax.lax.bitwise_and(t, NBUF - 1)

    def qslot(t):
        return t % NQ if st(t) else jax.lax.bitwise_and(t, NQ - 1)

    def when(cond, fn):
        if isinstance(cond, bool):
            if cond:
                fn()
        else:
            pl.when(cond)(fn)

    def land(a, b):
        if isinstance(a, bool) and isinstance(b, bool):
            return a and b
        return jnp.logical_and(a, b)

    def kv_start(hbm, buf, sem, t):
        sl = ring(t)
        src = hbm.at[bat(t), grp(t)]
        dst = buf.at[sl]
        seg = PW // NSEG
        for i in range(NSEG):
            lo = i * seg
            pltpu.make_async_copy(src.at[lo:lo + R0], dst.at[lo:lo + R0], sem.at[sl]).start(priority=HI)
            pltpu.make_async_copy(src.at[lo + R0:lo + seg], dst.at[lo + R0:lo + seg], sem.at[sl]).start(priority=LO)

    def kstart(t):
        kv_start(kt_hbm, kbuf, ksem, t)

    def vstart(t):
        kv_start(vt_hbm, vbuf, vsem, t)

    def wqcopy(g):
        return pltpu.make_async_copy(wq_hbm.at[:, g * PW:(g + 1) * PW], wqbuf.at[g], wqsem.at[g])

    def wocopy(g):
        return pltpu.make_async_copy(wo_hbm.at[g], wobuf.at[g], wosem.at[g])

    def wq_piece(g, i):
        rows = pl.ds(i * WQR, WQR) if st(i) else pl.ds(pl.multiple_of(i * WQR, 16), WQR)
        cols = pl.ds(g * PW, PW) if st(g) else pl.ds(pl.multiple_of(g * PW, 128), PW)
        return pltpu.make_async_copy(wq_hbm.at[rows, cols], wqbuf.at[g, rows], wqsem.at[g])

    def wo_piece(g, i):
        rows = pl.ds(i * WOR, WOR) if st(i) else pl.ds(pl.multiple_of(i * WOR, 16), WOR)
        return pltpu.make_async_copy(wo_hbm.at[g, rows], wobuf.at[g, rows], wosem.at[g])

    def xcopy(b):
        return pltpu.make_async_copy(x_hbm.at[b], xbuf.at[b], xsem.at[b])

    def ocopy(b):
        return pltpu.make_async_copy(obuf.at[b], out_hbm.at[b], osem.at[b])

    def arrival(buf, sem, idx):
        return pltpu.make_async_copy(buf.at[idx], buf.at[idx], sem.at[idx])

    lane = jax.lax.broadcasted_iota(jnp.int32, (SQ, 256), 1)

    def qproj(t):
        q = jnp.dot(xbuf[bat(t)], wqbuf[grp(t)], preferred_element_type=F32) * SCALE
        sl = qslot(t)
        qring[sl, 0] = jnp.where(lane < DH, q[:, 0:256], 0.0).astype(BF16)
        qring[sl, 1] = jnp.where(lane >= 64, q[:, 128:384], 0.0).astype(BF16)

    def qk(t, sl):
        ks = ring(t)
        qs = qslot(t)
        ss[sl][0] = jnp.dot(qring[qs, 0], kbuf[ks, 0:256, :], preferred_element_type=F32)
        ss[sl][1] = jnp.dot(qring[qs, 1], kbuf[ks, 128:384, :], preferred_element_type=F32)

    def softmax(sl):
        res = []
        for h in range(2):
            s = ss[sl][h]
            m = jnp.max(s, axis=-1, keepdims=True)
            p = jnp.exp2(s - m)
            l = jnp.sum(p, axis=-1, keepdims=True)
            res.append((p.astype(BF16), 1.0 / l))
        return res

    def pv(t, sl, res):
        vs = ring(t)
        (p0, r0), (p1, r1) = res
        ot0 = jax.lax.dot_general(vbuf[vs, 0:DH, :], p0, NT, preferred_element_type=F32)
        ot1 = jax.lax.dot_general(vbuf[vs, DH:PW, :], p1, NT, preferred_element_type=F32)
        o = jnp.concatenate([ot0, ot1], axis=0).T
        col = jax.lax.broadcasted_iota(jnp.int32, (SQ, PW), 1)
        oo[sl][...] = (o * jnp.where(col < DH, r0, r1)).astype(BF16)

    def outproj(t, sl, emit=False):
        b = bat(t)
        r = acc[b] + jnp.dot(oo[sl][...], wobuf[grp(t)], preferred_element_type=F32)
        if emit:
            obuf[b] = r.astype(BF16)
        if not (emit and st(t)):
            acc[b] = r

    def step(t, sl, do_qk=True, do_qp=True, emit=False):
        res = softmax(sl)
        if do_qk:
            qk(t + 1, 1 - sl)
        if do_qp:
            qproj(t + DQ)
        pv(t, sl, res)
        outproj(max(t - 1, 0) if st(t) else jnp.maximum(t - 1, 0), 1 - sl, emit)

    first_wq = B * (DQ // B + 1)
    assert 1 + DQ + WQ_LEAD <= first_wq and 1 + WO_LEAD <= B

    def issue(tk, tv):
        when(tk < T, lambda: kstart(tk))
        uq = tk + DQ + WQ_LEAD
        when(land(uq >= first_wq, uq < T), lambda: wq_piece(grp(uq), bat(uq)).start(priority=HI))
        when(tv < T, lambda: vstart(tv))
        uo = tk + WO_LEAD
        when(land(uo >= B, uo < T), lambda: wo_piece(grp(uo), bat(uo)).start(priority=HI))

    def refill(t):
        issue(t + 1 + PD, t + PD)

    def waits(t0, par, u, with_qp, align=2):
        todo = []

        def add(cond, buf, sem, idx):
            if cond is not False:
                todo.append((cond, arrival(buf, sem, idx)))
        for j in range(u):
            t = t0 + j
            add(not (st(t) and t + 1 >= T), kbuf, ksem, ring(t + 1))
            add(True, vbuf, vsem, ring(t))
        for j in range(u):
            t = t0 + j
            if with_qp and (par + j + DQ) % align == 0:
                add(bat(t + DQ) == 0, wqbuf, wqsem, grp(t + DQ))
            if (par + j - 1) % align == 0:
                add(bat(t - 1) == 0, wobuf, wosem, grp(t - 1))
        for c, cp in todo:
            when(c, cp.wait)

    xcopy(0).start(priority=HI)
    wqcopy(0).start(priority=HI)
    for xb in range(1, B):
        xcopy(xb).start(priority=LO)
    kstart(0)
    acc[...] = jnp.zeros_like(acc)
    o1[...] = jnp.zeros_like(o1)
    xcopy(0).wait()
    wqcopy(0).wait()
    issue(1, 0)
    qproj(0)
    for xb in range(1, XS):
        xcopy(xb).wait()
    for t in range(1, PD - 1):
        issue(t + 1, t)
    for t in range(1, XS):
        qproj(t)
    for xb in range(XS, B):
        xcopy(xb).wait()
    wqcopy(1).start(priority=HI)
    for t in range(XS, B):
        qproj(t)
    NGQ = DQ // B
    for g in range(1, NGQ):
        wqcopy(g).wait()
        if g == NGQ - 1:
            arrival(kbuf, ksem, 0).wait()
        wqcopy(g + 1).start(priority=HI)
        if g == 1:
            wocopy(0).start(priority=HI)
        for t in range(g * B, (g + 1) * B):
            qproj(t)
    qk(0, 0)
    issue(PD, PD - 1)

    t_light = T - DQ
    t_last = T - 2

    def run_block(t0, u, do_qp, emit=False):
        waits(t0, 0, u, do_qp, min(u, 8))
        for j in range(u):
            step(t0 + j, j % 2, do_qp=do_qp, emit=emit)
            refill(t0 + j)

    def heavy(i, c):
        run_block(i * UH, UH, True)
        return c

    assert t_light % UH == 0 and UH + 1 <= PD <= NBUF
    jax.lax.fori_loop(0, t_light // UH, heavy, 0)

    def light(i, c):
        run_block(t_light + i * UL, UL, False, True)
        return c

    assert (t_last - t_light) % UL == 0
    jax.lax.fori_loop(0, (t_last - t_light) // UL, light, 0)

    t0 = t_last
    waits(t0, 0, 2, False)
    for b in range(B - 3):
        ocopy(b).start(priority=HI)
    step(t0, 0, do_qp=False, emit=True)
    ocopy(B - 3).start(priority=HI)
    step(t0 + 1, 1, do_qk=False, do_qp=False, emit=True)
    ocopy(B - 2).start(priority=HI)
    outproj(T - 1, 1, True)
    ocopy(B - 1).start(priority=HI)
    for b in range(B):
        ocopy(b).wait()


@jax.jit
def pallas_standalone__mha_block_cached__near_ridge_kernel(x, k_cache, v_cache, wq, wo):
    kt = jnp.swapaxes(k_cache, 2, 3).reshape(B, NG, PW, SK)
    vt = jnp.swapaxes(v_cache, 2, 3).reshape(B, NG, PW, SK)
    wo3 = wo.reshape(NG, PW, D)
    return pl.pallas_call(
        _kernel,
        in_specs=[pl.BlockSpec(memory_space=pl.ANY)] * 5,
        out_specs=pl.BlockSpec(memory_space=pl.ANY),
        out_shape=jax.ShapeDtypeStruct((B, SQ, D), BF16),
        scratch_shapes=[
            pltpu.VMEM((B, SQ, D), BF16),
            pltpu.VMEM((NG, D, PW), BF16),
            pltpu.VMEM((NG, PW, D), BF16),
            pltpu.VMEM((NBUF, PW, SK), BF16),
            pltpu.VMEM((NBUF, PW, SK), BF16),
            pltpu.VMEM((NQ, 2, SQ, 256), BF16),
            pltpu.VMEM((2, SQ, SK), F32), pltpu.VMEM((2, SQ, SK), F32),
            pltpu.VMEM((SQ, PW), BF16), pltpu.VMEM((SQ, PW), BF16),
            pltpu.VMEM((B, SQ, D), F32),
            pltpu.VMEM((B, SQ, D), BF16),
            pltpu.SemaphoreType.DMA((NBUF,)),
            pltpu.SemaphoreType.DMA((NBUF,)),
            pltpu.SemaphoreType.DMA((NG,)),
            pltpu.SemaphoreType.DMA((NG,)),
            pltpu.SemaphoreType.DMA((B,)),
            pltpu.SemaphoreType.DMA((B,)),
        ],
        compiler_params=pltpu.CompilerParams(
            vmem_limit_bytes=64 * 1024 * 1024,
            disable_bounds_checks=True,
            disable_semaphore_checks=True,
        ),
    )(x, wq, kt, vt, wo3)
```
